```python
import jax
import jax.numpy as jnp

def _softmax(x, axis=-1):
    return jax.nn.softmax(x, axis=axis)

def _gelu(x):
    return jax.nn.gelu(x, approximate=True)

def _silu(x):
    return jax.nn.silu(x)

def _sigmoid(x):
    return jax.nn.sigmoid(x)

def _layernorm(x, axis=-1, eps=1e-05):
    m = jnp.mean(x, axis=axis, keepdims=True)
    v = jnp.var(x, axis=axis, keepdims=True)
    return (x - m) / jnp.sqrt(v + eps)

def _scatter_add(tgt, idx, src, axis=0):
    return tgt.at[idx].add(src)

def _segment_sum(src, seg, n):
    return jax.ops.segment_sum(src, seg, n)

class _Rng:

    def __init__(self, key):
        self._k = key

    def _next(self):
        self._k, sub = jax.random.split(self._k)
        return sub

    def normal(self, shape):
        return jax.random.normal(self._next(), shape, dtype=jnp.bfloat16)

    def randint(self, lo, hi, shape):
        return jax.random.randint(self._next(), shape, lo, hi, dtype=jnp.int32)

    def uniform(self, shape, lo=0.0, hi=1.0):
        return jax.random.uniform(self._next(), shape, jnp.bfloat16, lo, hi)

    def permutation(self, n):
        return jax.random.permutation(self._next(), n)
kernel_name = 'concat_heads__sliding_local_dilated__memory_aug_recurrent_mem_tr__prompt'

def setup_inputs():
    _rng = _Rng(jax.random.key(int.from_bytes(__import__("os").urandom(4), "little")))
    _w = lambda a: (lambda t: t.astype(jnp.bfloat16) if jnp.issubdtype(t.dtype, jnp.floating) else t)(jnp.asarray(a))

    def _A_setup():
        B, S, D = (1, 2048, 640)
        return {'x': _w((lambda *s: _rng.normal(s) * 0.05)(B, S, D)), 'wqkv': _w((lambda *s: _rng.normal(s) * 0.05)(D, 3 * D)), 'wo': _w((lambda *s: _rng.normal(s) * 0.05)(D, D))}
    _A_in = _A_setup()

    def _B_setup():
        B, S, Dm = (1, 2048, 640)
        H, Dh = (32, 192)
        M, seg = (8, 32)
        seg = min(seg, S)
        S = S // seg * seg
        return {'x': _w((lambda *s: _rng.normal(s) * 0.05)(B, S, Dm)), 'mem0': _w((lambda *s: _rng.normal(s) * 0.05)(B, M, Dm)), 'Wq': _w((lambda *s: _rng.normal(s) * 0.05)(Dm, H, Dh) * Dm ** (-0.5)), 'Wk': _w((lambda *s: _rng.normal(s) * 0.05)(Dm, H, Dh) * Dm ** (-0.5)), 'Wv': _w((lambda *s: _rng.normal(s) * 0.05)(Dm, H, Dh) * Dm ** (-0.5)), 'Wo': _w((lambda *s: _rng.normal(s) * 0.05)(H, Dh, Dm) * (H * Dh) ** (-0.5)), 'seg_len': seg}
    _B_in = _B_setup()
    return {'A_x': _A_in['x'], 'A_wqkv': _A_in['wqkv'], 'A_wo': _A_in['wo'], 'B_x': _B_in['x'], 'B_mem0': _B_in['mem0'], 'B_Wq': _B_in['Wq'], 'B_Wk': _B_in['Wk'], 'B_Wv': _B_in['Wv'], 'B_Wo': _B_in['Wo'], 'B_seg_len': _B_in['seg_len']}

def reference(A_x, A_wqkv, A_wo, B_x, B_mem0, B_Wq, B_Wk, B_Wv, B_Wo, B_seg_len):

    def _A_ref(x, wqkv, wo):
        B, S, D = x.shape
        H = 32
        Dh = D // H
        W, dil = (8, 2)
        qkv = (lambda x, *d: x.transpose(*d))((x @ wqkv).reshape(B, S, 3, H, Dh), 2, 0, 3, 1, 4)
        q, k, v = (qkv[0], qkv[1], qkv[2])
        scale = Dh ** (-0.5)
        pos = jnp.arange(S)
        off = jnp.arange(W) * dil
        idx = pos[:, None] - off[None, :]
        mask = idx >= 0
        idx_c = jnp.where(mask, idx, 0).reshape(-1)
        kg = k[:, :, idx_c, :].reshape(B, H, S, W, Dh)
        vg = v[:, :, idx_c, :].reshape(B, H, S, W, Dh)
        logits = jnp.einsum('bhsd,bhswd->bhsw', q, kg) * scale
        logits = jnp.where(mask[None, None, :, :], logits, -1000000000.0)
        attn = _softmax(logits, axis=-1)
        o = jnp.einsum('bhsw,bhswd->bhsd', attn, vg)
        return (lambda x, *d: x.transpose(*d))(o, 0, 2, 1, 3).reshape(B, S, D) @ wo

    def _B_ref(x, mem0, Wq, Wk, Wv, Wo, seg_len):
        B, S, Dm = x.shape
        H, Dh = (Wq.shape[1], Wq.shape[2])
        M = mem0.shape[1]
        scale = Dh ** (-0.5)
        n_seg = S // seg_len
        L = M + seg_len
        idx = jnp.arange(L)
        mask = (idx[:, None] < M) | (idx[:, None] >= idx[None, :])
        mem = mem0
        outs = []
        for s in range(n_seg):
            xs = x[:, s * seg_len:(s + 1) * seg_len, :].copy()
            h = jnp.concatenate([mem, xs], axis=1)
            q = jnp.einsum('btd,dhe->bhte', h, Wq)
            k = jnp.einsum('btd,dhe->bhte', h, Wk)
            v = jnp.einsum('btd,dhe->bhte', h, Wv)
            scores = jnp.einsum('bhqe,bhke->bhqk', q, k) * scale
            scores = jnp.where(mask[None, None], scores, -1000000000.0)
            p = _softmax(scores, axis=-1)
            o = jnp.einsum('bhqk,bhke->bhqe', p, v)
            o = jnp.einsum('bhte,hed->btd', o, Wo)
            mem = o[:, :M, :].copy()
            outs.append(o[:, M:, :])
        return jnp.concatenate(outs, axis=1)
    a = _A_ref(A_x, A_wqkv, A_wo)
    b = _B_ref(B_x, B_mem0, B_Wq, B_Wk, B_Wv, B_Wo, B_seg_len)
    return jnp.concatenate([a, b], axis=-1)
```

```python
import jax
import jax.numpy as jnp
from jax import lax
from jax.experimental import pallas as pl
from jax.experimental.pallas import tpu as pltpu

F32, BF16 = jnp.float32, jnp.bfloat16
NT = (((1,), (1,)), ((), ()))

S, D = 2048, 640
LT = D // 128
AH, AD, AW, ADIL = 32, 20, 8, 2
HALO = 16
H, DH, M, SEG = 32, 192, 8, 32
L = M + SEG
NP = H // 2
PW = 2 * DH


def _blockdiag(t):
    lane = lax.broadcasted_iota(jnp.int32, (L, 128), 1)
    z = jnp.zeros((L, 128), F32)
    t0, t1, t2 = t[:, 0:128], t[:, 128:256], t[:, 256:384]
    top = jnp.concatenate([t0, jnp.where(lane < 64, t1, 0.0), z], axis=1)
    bot = jnp.concatenate([z, jnp.where(lane >= 64, t1, 0.0), t2], axis=1)
    return jnp.concatenate([top, bot], axis=0).astype(BF16)


def _softmax_pair(sc):
    row = lax.broadcasted_iota(jnp.int32, (L, 2 * L), 0)
    col = lax.broadcasted_iota(jnp.int32, (L, 2 * L), 1)
    first = col < L
    key = jnp.where(first, col, col - L)
    ok = (row < M) | (row >= key)
    s = jnp.where(ok, sc * (DH ** -0.5), -1e9)
    m0 = jnp.max(jnp.where(first, s, -jnp.inf), axis=1, keepdims=True)
    m1 = jnp.max(jnp.where(first, -jnp.inf, s), axis=1, keepdims=True)
    e = jnp.exp(s - jnp.where(first, m0, m1))
    l0 = jnp.sum(jnp.where(first, e, 0.0), axis=1, keepdims=True)
    l1 = jnp.sum(jnp.where(first, 0.0, e), axis=1, keepdims=True)
    return e / jnp.where(first, l0, l1)


def make(lag1=2, lag2=4, ochunk=2, nseg=S // SEG, TB=128, RC=32, dma="all", ahead=3, OUTC=8):
    NB = S // TB

    def kern(ax_hbm, awqkv_hbm, awo_hbm, bx_hbm, mem_hbm, wq_hbm, wk_hbm, wv_hbm, wo_hbm,
             out_hbm,
             ax, awqkv, awo, tmp, wpt, wop, q_s, kv_s, oa_s, outa,
             bx, mem, raw, w3, wo, h_s, o_s, outb,
             sem_a, sem_w, sem_b, sem_o):
        cp = pltpu.make_async_copy
        c_wqkv = [cp(awqkv_hbm.at[:, pl.ds(j * D, D)], awqkv.at[j], sem_a.at[j]) for j in range(3)]
        c_ax = cp(ax_hbm, ax, sem_a.at[3])
        c_awo = cp(awo_hbm, awo, sem_a.at[4])
        c_w = [[cp(w.at[pl.ds(p * PW, PW), :], raw.at[p, j], sem_w.at[p, j])
                for j, w in enumerate((wq_hbm, wk_hbm, wv_hbm))] for p in range(NP)]
        c_bx = cp(bx_hbm, bx, sem_b.at[0])
        c_mem = cp(mem_hbm, mem, sem_b.at[1])
        c_wo = cp(wo_hbm, wo, sem_b.at[2])

        for c in c_wqkv:
            c.start()
        c_ax.start()
        c_awo.start()
        started = [0]

        def start_w(upto):
            while started[0] < min(upto, NP + 1):
                p = started[0]
                if p < NP:
                    for c in c_w[p]:
                        c.start()
                else:
                    c_mem.start()
                    c_bx.start()
                    c_wo.start()
                started[0] += 1

        if dma == "all":
            start_w(NP + 1)

        def permute_rows(dst, base):
            for d in range(AD):
                for t in range(LT):
                    dst[pl.ds(base + d * AH, AH), t * 128:(t + 1) * 128] = (
                        tmp[t, pl.ds(d, AH, stride=AD), :].astype(BF16))

        for j in range(3):
            c_wqkv[j].wait()
            for t in range(LT):
                tmp[t] = awqkv[j, t * 128:(t + 1) * 128, :].astype(F32).T
            permute_rows(wpt, j * D)
            if j == 0:
                start_w(1)
        c_awo.wait()
        for t in range(LT):
            tmp[t] = awo[:, t * 128:(t + 1) * 128].astype(F32)
        permute_rows(wop, 0)
        c_ax.wait()
        start_w(ahead)

        def a_proj(i, j):
            b = i % 2
            r = lax.dot_general(ax[i * TB:(i + 1) * TB, :], wpt[j * D:(j + 1) * D, :], NT,
                                preferred_element_type=F32)
            for t in range(LT):
                rt = r[:, t * 128:(t + 1) * 128]
                if j == 0:
                    q_s[b, t] = rt
                else:
                    c = (j - 1) * LT + t
                    kv_s[b, c, HALO:HALO + TB, :] = rt
                    if i == 0:
                        kv_s[b, c, 0:HALO, :] = jnp.broadcast_to(rt[0:1, :], (HALO, 128))
                    else:
                        kv_s[b, c, 0:HALO, :] = kv_s[1 - b, c, TB:TB + HALO, :]

        def a_attn(i, r0):
            b = i % 2
            q = [q_s[b, t, r0:r0 + RC, :] for t in range(LT)]
            lg = []
            for w in range(AW):
                lo = HALO + r0 - ADIL * w
                a = q[0] * kv_s[b, 0, lo:lo + RC, :]
                for t in range(1, LT):
                    a = a + q[t] * kv_s[b, t, lo:lo + RC, :]
                a = a + pltpu.roll(a, 64, 1)
                a = a + pltpu.roll(a, 32, 1)
                a = a * (AD ** -0.5)
                if i * TB + r0 < ADIL * w:
                    pos = lax.broadcasted_iota(jnp.int32, (RC, 128), 0) + (i * TB + r0)
                    a = jnp.where(pos >= ADIL * w, a, -1e9)
                lg.append(a)
            m = lg[0]
            for w in range(1, AW):
                m = jnp.maximum(m, lg[w])
            e = [jnp.exp(a - m) for a in lg]
            l = e[0]
            for w in range(1, AW):
                l = l + e[w]
            inv = 1.0 / l
            p = [x * inv for x in e]
            for t in range(LT):
                o = None
                for w in range(AW):
                    lo = HALO + r0 - ADIL * w
                    c = p[w] * kv_s[b, LT + t, lo:lo + RC, :]
                    o = c if o is None else o + c
                oa_s[b, r0:r0 + RC, t * 128:(t + 1) * 128] = o.astype(BF16)

        def a_out(i):
            r = jnp.dot(oa_s[i % 2], wop[...], preferred_element_type=F32)
            outa[i * TB:(i + 1) * TB, :] = r.astype(BF16)

        def w_prep(p, j):
            w3[p, :, j * PW:(j + 1) * PW] = raw[p, j].T

        nrc = TB // RC
        pps = NP // NB
        for i in range(NB + 2):
            ps = [p for p in range((i - 1) * pps, i * pps) if 0 <= p < NP]
            for p in ps:
                for c in c_w[p]:
                    c.wait()
            start_w(ahead + i * pps)
            chunks = list(range(nrc)) if 0 <= i - 1 < NB else []
            for j in range(4):
                if j < 3:
                    if i < NB:
                        a_proj(i, j)
                    for p in ps:
                        w_prep(p, j)
                elif 0 <= i - 2 < NB:
                    a_out(i - 2)
                for rc in chunks[j * nrc // 4:(j + 1) * nrc // 4]:
                    a_attn(i - 1, rc * RC)
        start_w(NP + 1)
        c_outa = cp(outa, out_hbm.at[:, pl.ds(0, D)], sem_o.at[0])
        c_outa.start()
        c_mem.wait()
        c_bx.wait()
        c_wo.wait()

        h_s[0:M, :] = mem[...].astype(F32)

        def step(s, carry):
            rows = pl.ds(pl.multiple_of(s * SEG, SEG), SEG)
            h_s[M:L, :] = bx[rows, :].astype(F32)
            st = {}

            def proj(p):
                qkv = jnp.dot(h_s[...], w3[p], preferred_element_type=F32)
                st[p] = dict(q=qkv[:, 0:PW], kb=_blockdiag(qkv[:, PW:2 * PW]),
                             vb=_blockdiag(qkv[:, 2 * PW:3 * PW]))

            def score(p):
                sc = lax.dot_general(st[p]["q"], st[p]["kb"], NT, preferred_element_type=F32)
                st[p]["p"] = _softmax_pair(sc)

            def pv(p):
                o_s[:, p * PW:(p + 1) * PW] = jnp.dot(st[p]["p"], st[p]["vb"], preferred_element_type=F32)

            acc = [None]

            def outp(ch):
                cs = slice(ch * ochunk * PW, (ch + 1) * ochunk * PW)
                r = jnp.dot(o_s[:, cs], wo[cs, :], preferred_element_type=F32)
                acc[0] = r if acc[0] is None else acc[0] + r

            nch = NP // ochunk
            done = 0
            for t in range(NP + lag2):
                if t < NP:
                    proj(t)
                if 0 <= t - lag1 < NP:
                    score(t - lag1)
                if t >= NP and done < nch - 1:
                    outp(done)
                    done += 1
                if 0 <= t - lag2 < NP:
                    pv(t - lag2)
            while done < nch:
                outp(done)
                done += 1
            out = acc[0]
            h_s[0:M, :] = out[0:M]
            outb[rows, :] = out[M:L].astype(BF16)
            return carry

        per = nseg // OUTC
        def group(g, carry):
            lax.fori_loop(g * per, (g + 1) * per, step, 0)
            r = pl.ds(pl.multiple_of(g * per * SEG, per * SEG), per * SEG)
            cp(outb.at[r, :], out_hbm.at[r, pl.ds(D, D)], sem_o.at[1]).start()
            return carry
        lax.fori_loop(0, OUTC, group, 0)
        c_outa.wait()
        r = pl.ds(0, nseg * SEG)
        cp(outb.at[r, :], out_hbm.at[r, pl.ds(D, D)], sem_o.at[1]).wait()

    V = pltpu.VMEM
    f = pl.pallas_call(
        kern,
        out_shape=jax.ShapeDtypeStruct((S, 2 * D), BF16),
        in_specs=[pl.BlockSpec(memory_space=pl.ANY)] * 9,
        out_specs=pl.BlockSpec(memory_space=pl.ANY),
        scratch_shapes=[
            V((S, D), BF16), V((3, D, D), BF16), V((D, D), BF16), V((LT, D, 128), F32),
            V((3 * D, D), BF16), V((D, D), BF16), V((2, LT, TB, 128), F32),
            V((2, 2 * LT, HALO + TB, 128), F32), V((2, TB, D), BF16), V((S, D), BF16),
            V((S, D), BF16), V((M, D), BF16), V((NP, 3, PW, D), BF16), V((NP, D, 3 * PW), BF16),
            V((H * DH, D), BF16), V((L, D), F32), V((L, H * DH), F32), V((S, D), BF16),
            pltpu.SemaphoreType.DMA((5,)), pltpu.SemaphoreType.DMA((NP, 3)),
            pltpu.SemaphoreType.DMA((3,)), pltpu.SemaphoreType.DMA((2,)),
        ],
        name="kf",
        compiler_params=pltpu.CompilerParams(vmem_limit_bytes=120 * 1024 * 1024))

    def fn(A_x, A_wqkv, A_wo, B_x, B_mem0, B_Wq, B_Wk, B_Wv, B_Wo):
        t = lambda w: w.transpose(1, 2, 0).reshape(H * DH, D)
        out = f(A_x.reshape(S, D), A_wqkv, A_wo, B_x.reshape(S, D), B_mem0.reshape(M, D),
                t(B_Wq), t(B_Wk), t(B_Wv), B_Wo.reshape(H * DH, D))
        return out.reshape(1, S, 2 * D)
    return fn


def pallas_concat_heads__sliding_local_dilated__memory_aug_recurrent_mem_tr__prompt_kernel(
    A_x, A_wqkv, A_wo, B_x, B_mem0, B_Wq, B_Wk, B_Wv, B_Wo, B_seg_len,
):
    assert B_seg_len == SEG
    return make(dma='chain')(A_x, A_wqkv, A_wo, B_x, B_mem0, B_Wq, B_Wk, B_Wv, B_Wo)
```

```python
import jax
import jax.numpy as jnp
from jax import lax
from jax.experimental import pallas as pl
from jax.experimental.pallas import tpu as pltpu

F32, BF16, U32 = jnp.float32, jnp.bfloat16, jnp.uint32
NT = (((1,), (1,)), ((), ()))

S, D = 2048, 640
LT = D // 128
AH, AD, AW, ADIL = 32, 20, 8, 2
HALO = 16
TB = 128
NB = S // TB
H, DH, M, SEG = 32, 192, 8, 32
L = M + SEG
NP = H // 2
PW = 2 * DH
NSEG = S // SEG


def _blockdiag(t):
    lane = lax.broadcasted_iota(jnp.int32, (L, 128), 1)
    z = jnp.zeros((L, 128), F32)
    t0, t1, t2 = t[:, 0:128], t[:, 128:256], t[:, 256:384]
    top = jnp.concatenate([t0, jnp.where(lane < 64, t1, 0.0), z], axis=1)
    bot = jnp.concatenate([z, jnp.where(lane >= 64, t1, 0.0), t2], axis=1)
    return jnp.concatenate([top, bot], axis=0).astype(BF16)


def _softmax_pair(sc):
    row = lax.broadcasted_iota(jnp.int32, (L, 2 * L), 0)
    col = lax.broadcasted_iota(jnp.int32, (L, 2 * L), 1)
    first = col < L
    key = jnp.where(first, col, col - L)
    ok = (row < M) | (row >= key)
    s = jnp.where(ok, sc * (DH ** -0.5), -1e9)
    m0 = jnp.max(jnp.where(first, s, -jnp.inf), axis=1, keepdims=True)
    m1 = jnp.max(jnp.where(first, -jnp.inf, s), axis=1, keepdims=True)
    e = jnp.exp(s - jnp.where(first, m0, m1))
    l0 = jnp.sum(jnp.where(first, e, 0.0), axis=1, keepdims=True)
    l1 = jnp.sum(jnp.where(first, 0.0, e), axis=1, keepdims=True)
    return e / jnp.where(first, l0, l1)


def make(lag1=2, lag2=4, ochunk=2, RC=16, ahead=6, UN=3, aorder=0, nit=None, WC=4, XC=4, omode="k", spl=(0, 3, 6, 8)):
    NIT = (NSEG - 1) // UN if nit is None else nit

    def kern(ax_hbm, awqkv_hbm, awo_hbm, bx_hbm, mem_hbm, wq_hbm, wk_hbm, wv_hbm, wo_hbm,
             out_hbm,
             ax, awqkv, awo, tmp, wpt, wop, q_s, kv_s, oa_s, outa,
             bx, mem, raw, w3, wo, h_s, o_s, outb,
             sem_a, sem_x, sem_w, sem_b, sem_wo, sem_o):
        cp = pltpu.make_async_copy
        XR = S // XC
        WR = H * DH // WC
        c_wqkv = [cp(awqkv_hbm.at[:, pl.ds(j * D, D)], awqkv.at[j], sem_a.at[j]) for j in range(3)]
        c_awo = cp(awo_hbm, awo, sem_a.at[3])
        c_ax = [cp(ax_hbm.at[pl.ds(c * XR, XR), :], ax.at[pl.ds(c * XR, XR), :], sem_x.at[c]) for c in range(XC)]

        def c_w(p):
            r = pl.ds(p * PW if isinstance(p, int) else pl.multiple_of(p * PW, PW), PW)
            return [cp(w.at[r, :], raw.at[p, j], sem_w.at[p, j]) for j, w in enumerate((wq_hbm, wk_hbm, wv_hbm))]

        c_mem = cp(mem_hbm, mem, sem_b.at[0])
        c_bx0 = cp(bx_hbm.at[pl.ds(0, SEG), :], bx.at[pl.ds(0, SEG), :], sem_b.at[1])
        c_bx1 = cp(bx_hbm.at[pl.ds(SEG, S - SEG), :], bx.at[pl.ds(SEG, S - SEG), :], sem_b.at[2])
        c_wo = [cp(wo_hbm.at[pl.ds(c * WR, WR), :], wo.at[pl.ds(c * WR, WR), :], sem_wo.at[c]) for c in range(WC)]

        c_wqkv[0].start()
        c_ax[0].start()
        c_wqkv[1].start()
        c_wqkv[2].start()
        c_awo.start()

        def permute_rows(dst, base):
            for d in range(AD):
                for t in range(LT):
                    dst[pl.ds((base + d * AH) // 2, AH // 2), t * 128:(t + 1) * 128] = pltpu.bitcast(
                        tmp[t, pl.ds(d, AH, stride=AD), :].astype(BF16), U32)

        def prep_qkv(j):
            for t in range(LT):
                tmp[t] = awqkv[j, t * 128:(t + 1) * 128, :].astype(F32).T
            permute_rows(wpt, j * D)

        def prep_wo():
            for t in range(LT):
                tmp[t] = awo[:, t * 128:(t + 1) * 128].astype(F32)
            permute_rows(wop, 0)

        def blk(i):
            return pl.ds(i * TB if isinstance(i, int) else pl.multiple_of(i * TB, TB), TB)

        def a_proj(i, b, j):
            w = pltpu.bitcast(wpt[j * D // 2:(j + 1) * D // 2, :], BF16)
            r = lax.dot_general(ax[blk(i), :], w, NT, preferred_element_type=F32)
            for t in range(LT):
                rt = r[:, t * 128:(t + 1) * 128]
                if j == 0:
                    q_s[b, t] = rt
                else:
                    c = (j - 1) * LT + t
                    kv_s[b, c, HALO:HALO + TB, :] = rt
                    if isinstance(i, int) and i == 0:
                        kv_s[b, c, 0:HALO, :] = jnp.broadcast_to(rt[0:1, :], (HALO, 128))
                    else:
                        kv_s[b, c, 0:HALO, :] = kv_s[1 - b, c, TB:TB + HALO, :]

        def a_attn(first, b, r0):
            q = [q_s[b, t, r0:r0 + RC, :] for t in range(LT)]
            lg = []
            for w in range(AW):
                lo = HALO + r0 - ADIL * w
                a = q[0] * kv_s[b, 0, lo:lo + RC, :]
                for t in range(1, LT):
                    a = a + q[t] * kv_s[b, t, lo:lo + RC, :]
                a = a + pltpu.roll(a, 64, 1)
                a = a + pltpu.roll(a, 32, 1)
                a = a * (AD ** -0.5)
                if first and r0 < ADIL * w:
                    pos = lax.broadcasted_iota(jnp.int32, (RC, 128), 0) + r0
                    a = jnp.where(pos >= ADIL * w, a, -1e9)
                lg.append(a)
            m = lg[0]
            for w in range(1, AW):
                m = jnp.maximum(m, lg[w])
            e = [jnp.exp(a - m) for a in lg]
            l = e[0]
            for w in range(1, AW):
                l = l + e[w]
            inv = 1.0 / l
            p = [x * inv for x in e]
            for t in range(LT):
                o = None
                for w in range(AW):
                    lo = HALO + r0 - ADIL * w
                    c = p[w] * kv_s[b, LT + t, lo:lo + RC, :]
                    o = c if o is None else o + c
                oa_s[b, r0:r0 + RC, t * 128:(t + 1) * 128] = o

        def a_out(i, b):
            r = jnp.dot(oa_s[b], pltpu.bitcast(wop[...], BF16), preferred_element_type=F32)
            outa[blk(i), :] = r.astype(BF16)

        def w_prep(p, j):
            w3[p, :, j * PW:(j + 1) * PW] = pltpu.bitcast(raw[p, j].T, U32)

        nrc = TB // RC
        splits = [(s * nrc) // 8 for s in spl]

        def stage(i, b, proj=True, attn=True, first=False, extra=()):
            for j in range(3):
                if j < len(extra):
                    extra[j]()
                if attn:
                    for rc in range(splits[j], splits[j + 1]):
                        a_attn(first, 1 - b, rc * RC)
                if proj:
                    a_proj(i, b, j)

        c_wqkv[0].wait()
        for c in c_ax[1:]:
            c.start()
        prep_qkv(0)
        c_ax[0].wait()
        c_wqkv[1].wait()
        for c in c_w(0):
            c.start()
        a_proj(0, 0, 0)
        prep_qkv(1)
        c_wqkv[2].wait()
        for c in c_w(1):
            c.start()
        a_proj(0, 0, 1)
        prep_qkv(2)
        a_proj(0, 0, 2)
        c_awo.wait()
        for p in range(2, ahead - 2):
            for c in c_w(p):
                c.start()
        prep_wo()
        stage(1, 1, first=True)
        a_out(0, 0)
        for c in c_ax[1:]:
            c.wait()

        def tail_dmas(k):
            if k == 0:
                c_mem.start()
                c_bx0.start()
            if k < WC:
                c_wo[k].start()
            if k == WC:
                c_bx1.start()

        nk = ahead // 2 - 1

        def a_iter(it, carry):
            i = 2 * it
            for c in c_w(i - 2) + c_w(i - 1):
                c.wait()
            nxt = i - 4 + ahead

            @pl.when(nxt < NP)
            def _():
                for c in c_w(nxt) + c_w(nxt + 1):
                    c.start()
            for k in range(nk - 1):
                @pl.when(nxt == NP + 2 * k)
                def _():
                    tail_dmas(2 * k)
                    tail_dmas(2 * k + 1)
            if aorder == 0:
                for j in range(3):
                    w_prep(i - 2, j)
                    w_prep(i - 1, j)
                stage(i, 0)
                stage(i + 1, 1)
            elif aorder == 1:
                stage(i, 0, extra=[lambda j=j: (w_prep(i - 2, j), w_prep(i - 1, j)) for j in range(3)])
                stage(i + 1, 1)
            else:
                stage(i, 0, extra=[lambda j=j: w_prep(i - 2, j) for j in range(3)])
                stage(i + 1, 1, extra=[lambda j=j: w_prep(i - 1, j) for j in range(3)])
            a_out(i - 1, 1)
            a_out(i, 0)
            return carry
        lax.fori_loop(1, NB // 2, a_iter, 0)
        for c in c_w(NP - 2) + c_w(NP - 1):
            c.wait()
        for k in range(2 * (nk - 1), WC + 1):
            tail_dmas(k)
        stage(NB, 0, proj=False)
        a_out(NB - 1, 1)
        for j in range(3):
            w_prep(NP - 2, j)
            w_prep(NP - 1, j)
        c_mem.wait()
        c_bx0.wait()

        def step(s, hb, before_out=None):
            rows = pl.ds(s * SEG if isinstance(s, int) else pl.multiple_of(s * SEG, SEG), SEG)
            h_s[hb, M:L, :] = bx[rows, :].astype(F32)
            st = {}

            def proj(p):
                qkv = jnp.dot(h_s[hb], pltpu.bitcast(w3[p], BF16), preferred_element_type=F32)
                st[p] = dict(q=qkv[:, 0:PW], kb=_blockdiag(qkv[:, PW:2 * PW]),
                             vb=_blockdiag(qkv[:, 2 * PW:3 * PW]))

            def score(p):
                sc = lax.dot_general(st[p]["q"], st[p]["kb"], NT, preferred_element_type=F32)
                st[p]["p"] = _softmax_pair(sc)

            def pv(p):
                o_s[:, p * PW:(p + 1) * PW] = jnp.dot(st[p]["p"], st[p]["vb"], preferred_element_type=F32)

            acc = [None]

            def outp(ch):
                if before_out is not None:
                    before_out(ch)
                cs = slice(ch * ochunk * PW, (ch + 1) * ochunk * PW)
                r = jnp.dot(o_s[:, cs], wo[cs, :], preferred_element_type=F32)
                acc[0] = r if acc[0] is None else acc[0] + r

            nch = NP // ochunk
            done = 0
            for t in range(NP + lag2):
                if t < NP:
                    proj(t)
                if 0 <= t - lag1 < NP:
                    score(t - lag1)
                if t >= NP and done < nch - 1 and before_out is None:
                    outp(done)
                    done += 1
                if 0 <= t - lag2 < NP:
                    pv(t - lag2)
            hn = (hb + 1) % UN if before_out is None else 0
            if omode == "k" or before_out is not None:
                while done < nch:
                    outp(done)
                    done += 1
                out = acc[0]
                h_s[hn, 0:M, :] = out[0:M]
                outb[rows, :] = out[M:L].astype(BF16)
            else:
                cs = slice(done * ochunk * PW, NP * PW)
                for n in range(LT):
                    ns = slice(n * 128, (n + 1) * 128)
                    out = acc[0][:, ns] + jnp.dot(o_s[:, cs], wo[cs, ns], preferred_element_type=F32)
                    h_s[hn, 0:M, ns] = out[0:M]
                    outb[rows, ns] = out[M:L].astype(BF16)

        h_s[0, 0:M, :] = mem[...].astype(F32)

        def wait_wo(ch):
            r0 = ch * ochunk * PW
            if r0 % WR == 0:
                c_wo[r0 // WR].wait()
        step(0, 0, wait_wo)
        c_bx1.wait()
        c_outa = cp(outa, out_hbm.at[:, pl.ds(0, D)], sem_o.at[0])
        c_outa.start()

        def c_outb(r0, n):
            r = pl.ds(r0, n)
            return cp(outb.at[r, :], out_hbm.at[r, pl.ds(D, D)], sem_o.at[1])
        c_outb(0, SEG).start()

        def b_iter(it, carry):
            s0 = 1 + it * UN
            for u in range(UN):
                step(s0 + u, u)
            c_outb(pl.multiple_of(s0 * SEG, SEG), UN * SEG).start()
            return carry
        lax.fori_loop(0, NIT, b_iter, 0)
        c_outa.wait()
        c_outb(0, SEG + NIT * UN * SEG).wait()

    V = pltpu.VMEM
    DMA = pltpu.SemaphoreType.DMA
    f = pl.pallas_call(
        kern,
        out_shape=jax.ShapeDtypeStruct((S, 2 * D), BF16),
        in_specs=[pl.BlockSpec(memory_space=pl.ANY)] * 9,
        out_specs=pl.BlockSpec(memory_space=pl.ANY),
        scratch_shapes=[
            V((S, D), BF16), V((3, D, D), BF16), V((D, D), BF16), V((LT, D, 128), F32),
            V((3 * D // 2, D), U32), V((D // 2, D), U32), V((2, LT, TB, 128), F32),
            V((2, 2 * LT, HALO + TB, 128), F32), V((2, TB, D), F32), V((S, D), BF16),
            V((S, D), BF16), V((M, D), BF16), V((NP, 3, PW, D), BF16), V((NP, D // 2, 3 * PW), U32),
            V((H * DH, D), BF16), V((UN, L, D), F32), V((L, H * DH), F32), V((S, D), BF16),
            DMA((4,)), DMA((XC,)), DMA((NP, 3)), DMA((3,)), DMA((WC,)), DMA((2,)),
        ],
        name="kf",
        compiler_params=pltpu.CompilerParams(vmem_limit_bytes=120 * 1024 * 1024))

    def fn(A_x, A_wqkv, A_wo, B_x, B_mem0, B_Wq, B_Wk, B_Wv, B_Wo):
        t = lambda w: w.transpose(1, 2, 0).reshape(H * DH, D)
        out = f(A_x.reshape(S, D), A_wqkv, A_wo, B_x.reshape(S, D), B_mem0.reshape(M, D),
                t(B_Wq), t(B_Wk), t(B_Wv), B_Wo.reshape(H * DH, D))
        return out.reshape(1, S, 2 * D)
    return fn


def pallas_concat_heads__sliding_local_dilated__memory_aug_recurrent_mem_tr__prompt_kernel(
    A_x, A_wqkv, A_wo, B_x, B_mem0, B_Wq, B_Wk, B_Wv, B_Wo, B_seg_len,
):
    assert B_seg_len == SEG
    return make(UN=3, aorder=1, RC=16, spl=[0, 4, 8, 8], ahead=8, omode='n')(A_x, A_wqkv, A_wo, B_x, B_mem0, B_Wq, B_Wk, B_Wv, B_Wo)
```

```python
import contextlib
import functools

import jax
import jax.numpy as jnp
from jax import lax
from jax.experimental import pallas as pl
from jax.experimental.pallas import tpu as pltpu

F32, BF16, U32 = jnp.float32, jnp.bfloat16, jnp.uint32
NT = (((1,), (1,)), ((), ()))

S, D = 2048, 640
LT = D // 128
AH, AD, AW, ADIL = 32, 20, 8, 2
HALO = 16
TB = 128
NB = S // TB
H, DH, M, SEG = 32, 192, 8, 32
L = M + SEG
NP = H // 2
PW = 2 * DH
NSEG = S // SEG


def _blockdiag(t):
    lane = lax.broadcasted_iota(jnp.int32, (L, 128), 1)
    z = jnp.zeros((L, 128), F32)
    t0, t1, t2 = t[:, 0:128], t[:, 128:256], t[:, 256:384]
    top = jnp.concatenate([t0, jnp.where(lane < 64, t1, 0.0), z], axis=1)
    bot = jnp.concatenate([z, jnp.where(lane >= 64, t1, 0.0), t2], axis=1)
    return jnp.concatenate([top, bot], axis=0).astype(BF16)


def _softmax_pair(sc):
    row = lax.broadcasted_iota(jnp.int32, (L, 2 * L), 0)
    col = lax.broadcasted_iota(jnp.int32, (L, 2 * L), 1)
    first = col < L
    key = jnp.where(first, col, col - L)
    ok = (row < M) | (row >= key)
    s = jnp.where(ok, sc * (DH ** -0.5), -1e9)
    m0 = jnp.max(jnp.where(first, s, -jnp.inf), axis=1, keepdims=True)
    m1 = jnp.max(jnp.where(first, -jnp.inf, s), axis=1, keepdims=True)
    e = jnp.exp(s - jnp.where(first, m0, m1))
    l0 = jnp.sum(jnp.where(first, e, 0.0), axis=1, keepdims=True)
    l1 = jnp.sum(jnp.where(first, 0.0, e), axis=1, keepdims=True)
    return e / jnp.where(first, l0, l1)


def make(lag1=2, lag2=4, ochunk=2, RC=16, UN=3, aorder=0, nit=None, WC=2, lag0=(2, 6), xp=False, xf=True, nl=6, w0=0, scopes=False, omode="k", PG=5, OG=5):
    NIT = (NSEG - 1) // UN if nit is None else nit

    def kern(ax_hbm, awqkv_hbm, awo_hbm, bx_hbm, mem_hbm, wq_hbm, wk_hbm, wv_hbm, wo_hbm,
             out_hbm,
             ax, awqkv, awo, tmp, wpt, wop, q_s, kv_s, oa_s, outa,
             bx, mem, raw, w3, wo, h_s, o_s, outb,
             sem_a, sem_x, sem_w, sem_b, sem_wo, sem_o):
        cp = pltpu.make_async_copy
        XO = (0, 2 * TB, 4 * TB, S)
        WR = H * DH // WC
        B1 = (1 + UN) * SEG

        def ds(i, n):
            return pl.ds(i * n if isinstance(i, int) else pl.multiple_of(i * n, n), n)

        c_wqkv = [cp(awqkv_hbm.at[:, pl.ds(j * D, D)], awqkv.at[j], sem_a.at[j]) for j in range(3)]
        c_awo = cp(awo_hbm, awo, sem_a.at[3])

        def c_ax(c):
            return cp(ax_hbm.at[pl.ds(XO[c], XO[c + 1] - XO[c]), :], ax.at[pl.ds(XO[c], XO[c + 1] - XO[c]), :], sem_x.at[c])

        def c_w(c):
            return [cp(w.at[ds(c, 2 * PW), :], raw.at[j, ds(c, 2 * PW), :], sem_w.at[c, j])
                    for j, w in enumerate((wq_hbm, wk_hbm, wv_hbm))]

        c_mem = cp(mem_hbm, mem, sem_b.at[0])
        c_bx0 = cp(bx_hbm.at[pl.ds(0, B1), :], bx.at[pl.ds(0, B1), :], sem_b.at[1])
        c_bx1 = cp(bx_hbm.at[pl.ds(B1, S - B1), :], bx.at[pl.ds(B1, S - B1), :], sem_b.at[2])
        c_wo = [cp(wo_hbm.at[ds(c, WR), :], wo.at[ds(c, WR), :], sem_wo.at[c]) for c in range(WC)]

        def start(cs):
            for c in cs:
                c.start()

        def wait(name, cs):
            with jax.named_scope(name) if scopes else contextlib.nullcontext():
                for c in cs:
                    c.wait()

        def permute_rows(dst, base):
            for d in range(AD):
                for t in range(LT):
                    dst[pl.ds((base + d * AH) // 2, AH // 2), t * 128:(t + 1) * 128] = pltpu.bitcast(
                        tmp[t, pl.ds(d, AH, stride=AD), :].astype(BF16), U32)

        def prep_qkv(j):
            for t in range(LT):
                tmp[t] = awqkv[j, t * 128:(t + 1) * 128, :].astype(F32).T
            permute_rows(wpt, j * D)

        def prep_wo():
            for t in range(LT):
                tmp[t] = awo[:, t * 128:(t + 1) * 128].astype(F32)
            permute_rows(wop, 0)

        def blk(i):
            return pl.ds(i * TB if isinstance(i, int) else pl.multiple_of(i * TB, TB), TB)

        def a_proj(i, b, c0, c1):
            w = pltpu.bitcast(wpt[c0 * 64:c1 * 64, :], BF16)
            r = lax.dot_general(ax[blk(i), :].astype(F32) if xf else ax[blk(i), :], w, NT, preferred_element_type=F32)
            for c in range(c0, c1):
                rt = r[:, (c - c0) * 128:(c - c0 + 1) * 128]
                if c < LT:
                    q_s[b, c] = rt
                else:
                    kv_s[b, c - LT, HALO:HALO + TB, :] = rt
                    if isinstance(i, int) and i == 0:
                        kv_s[b, c - LT, 0:HALO, :] = jnp.broadcast_to(rt[0:1, :], (HALO, 128))
                    else:
                        kv_s[b, c - LT, 0:HALO, :] = kv_s[1 - b, c - LT, TB:TB + HALO, :]

        def attn_tasks(b, first=False):
            st = {}

            def logits(r0):
                q = [q_s[b, t, r0:r0 + RC, :] for t in range(LT)]
                lg = []
                for w in range(AW):
                    lo = HALO + r0 - ADIL * w
                    a = q[0] * kv_s[b, 0, lo:lo + RC, :]
                    for t in range(1, LT):
                        a = a + q[t] * kv_s[b, t, lo:lo + RC, :]
                    lg.append(a + pltpu.roll(a, 64, 1))
                st[r0] = lg

            def fold(r0):
                st[r0] = [a + pltpu.roll(a, 32, 1) for a in st[r0]]

            def soft(r0):
                lg = []
                for w, a in enumerate(st[r0]):
                    a = a * (AD ** -0.5)
                    if first and r0 < ADIL * w:
                        pos = lax.broadcasted_iota(jnp.int32, (RC, 128), 0) + r0
                        a = jnp.where(pos >= ADIL * w, a, -1e9)
                    lg.append(a)
                m = lg[0]
                for w in range(1, AW):
                    m = jnp.maximum(m, lg[w])
                e = [jnp.exp(a - m) for a in lg]
                l = e[0]
                for w in range(1, AW):
                    l = l + e[w]
                inv = 1.0 / l
                st[r0] = [x * inv for x in e]

            def mix(r0):
                p = st.pop(r0)
                for t in range(LT):
                    o = None
                    for w in range(AW):
                        lo = HALO + r0 - ADIL * w
                        c = p[w] * kv_s[b, LT + t, lo:lo + RC, :]
                        o = c if o is None else o + c
                    oa_s[b, r0:r0 + RC, t * 128:(t + 1) * 128] = o

            return [functools.partial(f, r0) for r0 in range(0, TB, RC) for f in (logits, fold, soft, mix)]

        def a_out(i, b, c0, c1):
            ns = slice(c0 * 128, c1 * 128)
            r = jnp.dot(oa_s[b], pltpu.bitcast(wop[:, ns], BF16), preferred_element_type=F32)
            outa[blk(i), ns] = r.astype(BF16)

        def w_prep(p, j):
            w3[p, :, j * PW:(j + 1) * PW] = pltpu.bitcast(raw[j, ds(p, PW), :].T, U32)

        def proj_tasks(i, b, lo=0, hi=3 * LT):
            return [functools.partial(a_proj, i, b, c, min(c + PG, hi)) for c in range(lo, hi, PG)]

        def out_tasks(i, b):
            return [functools.partial(a_out, i, b, c, min(c + OG, LT)) for c in range(0, LT, OG)]

        def prep_tasks(p):
            return [functools.partial(w_prep, p, j) for j in range(3)]

        def run(*lists):
            keyed = [((k + off) / len(l), n, t) for n, (l, off) in enumerate(lists) if l for k, t in enumerate(l)]
            for _, _, t in sorted(keyed, key=lambda e: e[:2]):
                t()

        def a_body(i, preps, mid=None):
            pr = [prep_tasks(p) for p in preps]
            if aorder >= 2:
                flat = [x[j] for j in range(3) for x in pr]
                for b in range(2):
                    mine = flat[3 * b:3 * b + 3]
                    if aorder == 2:
                        run((proj_tasks(i + b, b), 0), (attn_tasks(1 - b), 0))
                        run((out_tasks(i + b - 1, 1 - b), 0), (mine, 0))
                    elif aorder == 3:
                        run((proj_tasks(i + b, b), 0), (attn_tasks(1 - b), 0), (mine, 0))
                        run((out_tasks(i + b - 1, 1 - b), 0))
                    else:
                        run((proj_tasks(i + b, b), 0), (attn_tasks(1 - b) + mine, 0))
                        run((out_tasks(i + b - 1, 1 - b), 0))
                    if b == 0 and mid is not None:
                        mid()
                return
            if aorder == 0:
                for b in range(2):
                    at, pj = attn_tasks(1 - b), proj_tasks(i + b, b)
                    for j in range(3):
                        for t in ([x[j] for x in pr] if b == 0 else []) + at[j * len(at) // 2:(j + 1) * len(at) // 2]:
                            t()
                        for t in pj[j * len(pj) // 3:(j + 1) * len(pj) // 3]:
                            t()
                run((out_tasks(i - 1, 1) + out_tasks(i, 0), 0))
            else:
                run((proj_tasks(i, 0), 0), (attn_tasks(1), 0), ([t for x in pr for t in x], 0))
                run((proj_tasks(i + 1, 1) + out_tasks(i - 1, 1), 0), (attn_tasks(0), 0))
                run((out_tasks(i, 0), 0))

        start([c_wqkv[0], c_ax(0), c_wqkv[1]])
        wait("zw0", [c_wqkv[0]])
        start([c_wqkv[2]])
        prep_qkv(0)
        wait("zw1", [c_ax(0), c_wqkv[1]])
        start([c_awo, c_ax(1)])
        run((proj_tasks(0, 0, 0, LT), 0))
        prep_qkv(1)
        wait("zw2", [c_wqkv[2]])
        start([c_ax(2)])
        run((proj_tasks(0, 0, LT, 2 * LT), 0))
        prep_qkv(2)
        run((proj_tasks(0, 0, 2 * LT, 3 * LT), 0))
        wait("zw3", [c_awo])
        start(c_w(0))
        prep_wo()
        run((proj_tasks(1, 1), 0), (attn_tasks(0, True), 0))
        run((out_tasks(0, 0), 0))
        start(c_w(1))

        def a_iter(it, carry):
            c = jnp.where(it == 1, NP // 2 - 1, it - 2)

            @pl.when(it == 1)
            def _():
                wait("zw4", [c_ax(1)])

            @pl.when(it > 1)
            def _():
                @pl.when(it + 1 < NP // 2)
                def _():
                    start(c_w(it + 1))
                for k in range(WC):
                    @pl.when(it == NB // 2 - WC + k)
                    def _():
                        start(([c_mem, c_bx0] if k == 0 else []) + [c_wo[k]])
                wait("zwl", c_w(c))

            def mid():
                @pl.when(it == 1)
                def _():
                    wait("zw4", [c_ax(2)])
                    start(c_w(2))
            a_body(2 * it, [2 * c, 2 * c + 1], mid)
            return carry
        lax.fori_loop(1, NB // 2, a_iter, 0)
        PD = NP - 4
        wait("zw5", c_w(NB // 2 - 2) + c_w(NB // 2 - 1) + [c_mem, c_bx0])
        late = attn_tasks(1)
        late_w = [t for p in range(PD, NP) for t in prep_tasks(p)]

        def step(s, hb, before_out=None):
            rows = pl.ds(s * SEG if isinstance(s, int) else pl.multiple_of(s * SEG, SEG), SEG)
            h_s[hb, M:L, :] = bx[rows, :].astype(F32)
            st = {}

            def proj(p, from_raw=False):
                if from_raw:
                    w = jnp.concatenate([raw[j, ds(p, PW), :] for j in range(3)], axis=0)
                    qkv = lax.dot_general(h_s[hb], w, NT, preferred_element_type=F32)
                else:
                    qkv = jnp.dot(h_s[hb], pltpu.bitcast(w3[p], BF16), preferred_element_type=F32)
                st[p] = dict(q=qkv[:, 0:PW], kb=_blockdiag(qkv[:, PW:2 * PW]),
                             vb=_blockdiag(qkv[:, 2 * PW:3 * PW]))

            def score(p):
                sc = lax.dot_general(st[p]["q"], st[p]["kb"], NT, preferred_element_type=F32)
                st[p]["p"] = _softmax_pair(sc)

            def pv(p):
                o_s[:, p * PW:(p + 1) * PW] = jnp.dot(st[p]["p"], st[p]["vb"], preferred_element_type=F32)

            acc = [None]

            def outp(ch):
                if before_out is not None:
                    before_out(ch)
                cs = slice(ch * ochunk * PW, (ch + 1) * ochunk * PW)
                r = jnp.dot(o_s[:, cs], wo[cs, :], preferred_element_type=F32)
                acc[0] = r if acc[0] is None else acc[0] + r

            nch = NP // ochunk
            done = 0
            fst = before_out is not None
            l1, l2 = (lag1, lag2) if not fst else lag0
            for t in range(NP + l2):
                if t < NP:
                    if fst and xp and t >= PD:
                        proj(t, True)
                    else:
                        proj(t)
                if fst:
                    for task in late[t * len(late) // nl:(t + 1) * len(late) // nl]:
                        task()
                    if not xp and t >= w0:
                        u = t - w0
                        for task in late_w[u * len(late_w) // (PD - w0):(u + 1) * len(late_w) // (PD - w0)]:
                            task()
                if 0 <= t - l1 < NP:
                    score(t - l1)
                if t >= NP and done < nch - 1 and not fst:
                    outp(done)
                    done += 1
                if fst and t >= NP:
                    ot = out_tasks(NB - 1, 1)
                    for task in ot[(t - NP) * len(ot) // l2:(t - NP + 1) * len(ot) // l2]:
                        task()
                if 0 <= t - l2 < NP:
                    pv(t - l2)
            if fst and xp:
                for task in late_w:
                    task()
            hn = (hb + 1) % UN if before_out is None else 0
            if omode == "k" or before_out is not None:
                while done < nch:
                    outp(done)
                    done += 1
                out = acc[0]
                h_s[hn, 0:M, :] = out[0:M]
                outb[rows, :] = out[M:L].astype(BF16)
            else:
                cs = slice(done * ochunk * PW, NP * PW)
                for n in range(LT):
                    ns = slice(n * 128, (n + 1) * 128)
                    out = acc[0][:, ns] + jnp.dot(o_s[:, cs], wo[cs, ns], preferred_element_type=F32)
                    h_s[hn, 0:M, ns] = out[0:M]
                    outb[rows, ns] = out[M:L].astype(BF16)

        h_s[0, 0:M, :] = mem[...].astype(F32)

        def wait_wo(ch):
            r0 = ch * ochunk * PW
            if r0 == 0:
                wait("zwo", c_wo)
                c_bx1.start()
        step(0, 0, wait_wo)
        c_outa = cp(outa, out_hbm.at[:, pl.ds(0, D)], sem_o.at[0])
        c_outa.start()

        def c_outb(r0, n):
            r = pl.ds(r0, n)
            return cp(outb.at[r, :], out_hbm.at[r, pl.ds(D, D)], sem_o.at[1])
        c_outb(0, SEG).start()

        def b_iter(it, carry):
            s0 = 1 + it * UN

            @pl.when(it == 1)
            def _():
                c_bx1.wait()
            for u in range(UN):
                step(s0 + u, u)
            c_outb(pl.multiple_of(s0 * SEG, SEG), UN * SEG).start()
            return carry
        lax.fori_loop(0, NIT, b_iter, 0)
        wait("zend", [c_outa, c_outb(0, SEG + NIT * UN * SEG)])

    V = pltpu.VMEM
    DMA = pltpu.SemaphoreType.DMA
    f = pl.pallas_call(
        kern,
        out_shape=jax.ShapeDtypeStruct((S, 2 * D), BF16),
        in_specs=[pl.BlockSpec(memory_space=pl.ANY)] * 9,
        out_specs=pl.BlockSpec(memory_space=pl.ANY),
        scratch_shapes=[
            V((S, D), BF16), V((3, D, D), BF16), V((D, D), BF16), V((LT, D, 128), F32),
            V((3 * D // 2, D), U32), V((D // 2, D), U32), V((2, LT, TB, 128), F32),
            V((2, 2 * LT, HALO + TB, 128), F32), V((2, TB, D), F32), V((S, D), BF16),
            V((S, D), BF16), V((M, D), BF16), V((3, H * DH, D), BF16), V((NP, D // 2, 3 * PW), U32),
            V((H * DH, D), BF16), V((UN, L, D), F32), V((L, H * DH), F32), V((S, D), BF16),
            DMA((4,)), DMA((3,)), DMA((NP // 2, 3)), DMA((3,)), DMA((WC,)), DMA((2,)),
        ],
        name="kf",
        compiler_params=pltpu.CompilerParams(vmem_limit_bytes=120 * 1024 * 1024))

    def fn(A_x, A_wqkv, A_wo, B_x, B_mem0, B_Wq, B_Wk, B_Wv, B_Wo):
        t = lambda w: w.transpose(1, 2, 0).reshape(H * DH, D)
        out = f(A_x.reshape(S, D), A_wqkv, A_wo, B_x.reshape(S, D), B_mem0.reshape(M, D),
                t(B_Wq), t(B_Wk), t(B_Wv), B_Wo.reshape(H * DH, D))
        return out.reshape(1, S, 2 * D)
    return fn


def pallas_concat_heads__sliding_local_dilated__memory_aug_recurrent_mem_tr__prompt_kernel(
    A_x, A_wqkv, A_wo, B_x, B_mem0, B_Wq, B_Wk, B_Wv, B_Wo, B_seg_len,
):
    assert B_seg_len == SEG
    return make(UN=3, omode='n', aorder=4, xf=False)(A_x, A_wqkv, A_wo, B_x, B_mem0, B_Wq, B_Wk, B_Wv, B_Wo)
```

```python
import contextlib
import functools

import jax
import jax.numpy as jnp
from jax import lax
from jax.experimental import pallas as pl
from jax.experimental.pallas import tpu as pltpu

F32, BF16, U32 = jnp.float32, jnp.bfloat16, jnp.uint32
NT = (((1,), (1,)), ((), ()))

S, D = 2048, 640
LT = D // 128
AH, AD, AW, ADIL = 32, 20, 8, 2
HALO = 16
TB = 128
NB = S // TB
H, DH, M, SEG = 32, 192, 8, 32
L = M + SEG
NP = H // 2
PW = 2 * DH
NSEG = S // SEG


def _blockdiag(t):
    lane = lax.broadcasted_iota(jnp.int32, (L, 128), 1)
    z = jnp.zeros((L, 128), F32)
    t0, t1, t2 = t[:, 0:128], t[:, 128:256], t[:, 256:384]
    top = jnp.concatenate([t0, jnp.where(lane < 64, t1, 0.0), z], axis=1)
    bot = jnp.concatenate([z, jnp.where(lane >= 64, t1, 0.0), t2], axis=1)
    return jnp.concatenate([top, bot], axis=0).astype(BF16)


def _softmax_pair(sc):
    row = lax.broadcasted_iota(jnp.int32, (L, 2 * L), 0)
    col = lax.broadcasted_iota(jnp.int32, (L, 2 * L), 1)
    first = col < L
    key = jnp.where(first, col, col - L)
    ok = (row < M) | (row >= key)
    s = jnp.where(ok, sc * (DH ** -0.5), -1e9)
    m0 = jnp.max(jnp.where(first, s, -jnp.inf), axis=1, keepdims=True)
    m1 = jnp.max(jnp.where(first, -jnp.inf, s), axis=1, keepdims=True)
    e = jnp.exp(s - jnp.where(first, m0, m1))
    l0 = jnp.sum(jnp.where(first, e, 0.0), axis=1, keepdims=True)
    l1 = jnp.sum(jnp.where(first, 0.0, e), axis=1, keepdims=True)
    return e / jnp.where(first, l0, l1)


def make(lag1=2, lag2=4, ochunk=2, RC=8, UN=3, aorder=4, nit=None, WC=4, wos=(0, 0, 2), lag0=(2, 6), xp=False, sk=(0, 1, 2, 2), fl=2, xf=False, nl=6, w0=0, scopes=False, omode="k", PG=5, OG=5):
    NIT = (NSEG - 1) // UN if nit is None else nit

    def kern(ax_hbm, awqkv_hbm, awo_hbm, bx_hbm, mem_hbm, wq_hbm, wk_hbm, wv_hbm, wo_hbm,
             out_hbm,
             ax, awqkv, awo, tmp, wpt, wop, q_s, kv_s, oa_s, outa,
             bx, mem, raw, w3, wo, h_s, o_s, outb,
             sem_a, sem_x, sem_w, sem_b, sem_wo, sem_o, *fens):
        cp = pltpu.make_async_copy
        XO = (0, 2 * TB, 4 * TB, S)
        WR = H * DH // WC
        B1 = (1 + UN) * SEG

        def ds(i, n):
            return pl.ds(i * n if isinstance(i, int) else pl.multiple_of(i * n, n), n)

        c_wqkv = [cp(awqkv_hbm.at[:, pl.ds(j * D, D)], awqkv.at[j], sem_a.at[j]) for j in range(3)]
        c_awo = cp(awo_hbm, awo, sem_a.at[3])

        def c_ax(c):
            return cp(ax_hbm.at[pl.ds(XO[c], XO[c + 1] - XO[c]), :], ax.at[pl.ds(XO[c], XO[c + 1] - XO[c]), :], sem_x.at[c])

        def c_w(c):
            return [cp(w.at[ds(c, 2 * PW), :], raw.at[j, ds(c, 2 * PW), :], sem_w.at[c, j])
                    for j, w in enumerate((wq_hbm, wk_hbm, wv_hbm))]

        c_mem = cp(mem_hbm, mem, sem_b.at[0])
        c_bx0 = cp(bx_hbm.at[pl.ds(0, B1), :], bx.at[pl.ds(0, B1), :], sem_b.at[1])
        c_bx1 = cp(bx_hbm.at[pl.ds(B1, S - B1), :], bx.at[pl.ds(B1, S - B1), :], sem_b.at[2])
        c_wo = [cp(wo_hbm.at[ds(c, WR), :], wo.at[ds(c, WR), :], sem_wo.at[c]) for c in range(WC)]

        def start(cs):
            for c in cs:
                c.start()

        def wait(name, cs):
            with jax.named_scope(name) if scopes else contextlib.nullcontext():
                for c in cs:
                    c.wait()

        def permute_rows(dst, base):
            for d in range(AD):
                for t in range(LT):
                    dst[pl.ds((base + d * AH) // 2, AH // 2), t * 128:(t + 1) * 128] = pltpu.bitcast(
                        tmp[t, pl.ds(d, AH, stride=AD), :].astype(BF16), U32)

        def prep_qkv(j):
            for t in range(LT):
                tmp[t] = awqkv[j, t * 128:(t + 1) * 128, :].astype(F32).T
            permute_rows(wpt, j * D)

        def prep_wo():
            for t in range(LT):
                tmp[t] = awo[:, t * 128:(t + 1) * 128].astype(F32)
            permute_rows(wop, 0)

        def blk(i):
            return pl.ds(i * TB if isinstance(i, int) else pl.multiple_of(i * TB, TB), TB)

        def a_proj(i, b, c0, c1, fen=None):
            w = pltpu.bitcast(wpt[c0 * 64:c1 * 64, :], BF16)
            x = ax[blk(i), :]
            if fen is not None:
                fen[0:8, :] = pltpu.bitcast(x[0:16, 0:128], F32)
                zero = pl.multiple_of(lax.shift_right_logical(i, 16) * 8, 8)
                x00 = pltpu.bitcast(fen[pl.ds(zero, 8), :], BF16)
                x = jnp.concatenate([jnp.concatenate([x00, x[0:16, 128:]], axis=1), x[16:]], axis=0)
            r = lax.dot_general(x.astype(F32) if xf else x, w, NT, preferred_element_type=F32)
            for c in range(c0, c1):
                rt = r[:, (c - c0) * 128:(c - c0 + 1) * 128]
                if c < LT:
                    q_s[b, c] = rt
                else:
                    kv_s[b, c - LT, HALO:HALO + TB, :] = rt
                    if isinstance(i, int) and i == 0:
                        kv_s[b, c - LT, 0:HALO, :] = jnp.broadcast_to(rt[0:1, :], (HALO, 128))
                    else:
                        kv_s[b, c - LT, 0:HALO, :] = kv_s[1 - b, c - LT, TB:TB + HALO, :]

        def attn_tasks(b, first=False, fenced=False):
            st = {}

            def logits(r0):
                q = [q_s[b, t, r0:r0 + RC, :] for t in range(LT)]
                lg = []
                for w in range(AW):
                    lo = HALO + r0 - ADIL * w
                    a = q[0] * kv_s[b, 0, lo:lo + RC, :]
                    for t in range(1, LT):
                        a = a + q[t] * kv_s[b, t, lo:lo + RC, :]
                    lg.append(a + pltpu.roll(a, 64, 1))
                st[r0] = lg

            def fold(r0):
                st[r0] = [a + pltpu.roll(a, 32, 1) for a in st[r0]]

            def soft(r0):
                lg = []
                for w, a in enumerate(st[r0]):
                    a = a * (AD ** -0.5)
                    if first and r0 < ADIL * w:
                        pos = lax.broadcasted_iota(jnp.int32, (RC, 128), 0) + r0
                        a = jnp.where(pos >= ADIL * w, a, -1e9)
                    lg.append(a)
                m = lg[0]
                for w in range(1, AW):
                    m = jnp.maximum(m, lg[w])
                e = [jnp.exp(a - m) for a in lg]
                l = e[0]
                for w in range(1, AW):
                    l = l + e[w]
                inv = 1.0 / l
                st[r0] = [x * inv for x in e]

            def mix(r0):
                p = st.pop(r0)
                for t in range(LT):
                    o = None
                    for w in range(AW):
                        lo = HALO + r0 - ADIL * w
                        c = p[w] * kv_s[b, LT + t, lo:lo + RC, :]
                        o = c if o is None else o + c
                    oa_s[b, r0:r0 + RC, t * 128:(t + 1) * 128] = o
                    if fenced:
                        fens[(r0 // RC) % len(fens)][8 + t * RC:8 + (t + 1) * RC, :] = o

            n = TB // RC
            return [functools.partial(f, (t - d) * RC) for t in range(n + max(sk))
                    for f, d in zip((logits, fold, soft, mix), sk) if 0 <= t - d < n]

        def a_out(i, b, c0, c1):
            ns = slice(c0 * 128, c1 * 128)
            r = jnp.dot(oa_s[b], pltpu.bitcast(wop[:, ns], BF16), preferred_element_type=F32)
            outa[blk(i), ns] = r.astype(BF16)

        def w_prep(p, j):
            w3[p, :, j * PW:(j + 1) * PW] = pltpu.bitcast(raw[j, ds(p, PW), :].T, U32)

        def proj_tasks(i, b, lo=0, hi=3 * LT):
            return [functools.partial(a_proj, i, b, c, min(c + PG, hi)) for c in range(lo, hi, PG)]

        def out_tasks(i, b):
            return [functools.partial(a_out, i, b, c, min(c + OG, LT)) for c in range(0, LT, OG)]

        def prep_tasks(p):
            return [functools.partial(w_prep, p, j) for j in range(3)]

        def run(*lists):
            keyed = [((k + off) / len(l), n, t) for n, (l, off) in enumerate(lists) if l for k, t in enumerate(l)]
            for _, _, t in sorted(keyed, key=lambda e: e[:2]):
                t()

        def a_body(i, preps, mid=None):
            pr = [prep_tasks(p) for p in preps]
            if aorder >= 2:
                flat = [x[j] for j in range(3) for x in pr]
                for b in range(2):
                    mine = flat[3 * b:3 * b + 3]
                    if aorder >= 5:
                        at = attn_tasks(1 - b, fenced=True)
                        cs = list(range(0, 3 * LT, PG))
                        nc = TB // RC
                        for n, c in enumerate(cs):
                            k = (n * nc) // len(cs) - fl
                            a_proj(i + b, b, c, min(c + PG, 3 * LT), fens[k % len(fens)] if k >= 0 else None)
                            for task in at[4 * ((n * nc) // len(cs)):4 * (((n + 1) * nc) // len(cs))]:
                                task()
                            if aorder == 5:
                                for task in mine[(n * len(mine)) // len(cs):((n + 1) * len(mine)) // len(cs)]:
                                    task()
                        run((out_tasks(i + b - 1, 1 - b), 0), (mine if aorder == 6 else [], 0))
                    elif aorder == 2:
                        run((proj_tasks(i + b, b), 0), (attn_tasks(1 - b), 0))
                        run((out_tasks(i + b - 1, 1 - b), 0), (mine, 0))
                    elif aorder == 3:
                        run((proj_tasks(i + b, b), 0), (attn_tasks(1 - b), 0), (mine, 0))
                        run((out_tasks(i + b - 1, 1 - b), 0))
                    else:
                        run((proj_tasks(i + b, b), 0), (attn_tasks(1 - b) + mine, 0))
                        run((out_tasks(i + b - 1, 1 - b), 0))
                    if b == 0 and mid is not None:
                        mid()
                return
            if aorder == 0:
                for b in range(2):
                    at, pj = attn_tasks(1 - b), proj_tasks(i + b, b)
                    for j in range(3):
                        for t in ([x[j] for x in pr] if b == 0 else []) + at[j * len(at) // 2:(j + 1) * len(at) // 2]:
                            t()
                        for t in pj[j * len(pj) // 3:(j + 1) * len(pj) // 3]:
                            t()
                run((out_tasks(i - 1, 1) + out_tasks(i, 0), 0))
            else:
                run((proj_tasks(i, 0), 0), (attn_tasks(1), 0), ([t for x in pr for t in x], 0))
                run((proj_tasks(i + 1, 1) + out_tasks(i - 1, 1), 0), (attn_tasks(0), 0))
                run((out_tasks(i, 0), 0))

        start([c_wqkv[0], c_ax(0), c_wqkv[1]])
        wait("zw0", [c_wqkv[0]])
        start([c_wqkv[2]])
        prep_qkv(0)
        wait("zw1", [c_ax(0), c_wqkv[1]])
        start([c_awo, c_ax(1)])
        run((proj_tasks(0, 0, 0, LT), 0))
        prep_qkv(1)
        wait("zw2", [c_wqkv[2]])
        start([c_ax(2)])
        run((proj_tasks(0, 0, LT, 2 * LT), 0))
        prep_qkv(2)
        run((proj_tasks(0, 0, 2 * LT, 3 * LT), 0))
        wait("zw3", [c_awo])
        start(c_w(0))
        prep_wo()
        run((proj_tasks(1, 1), 0), (attn_tasks(0, True), 0))
        run((out_tasks(0, 0), 0))
        start(c_w(1))

        def a_iter(it, carry):
            c = jnp.where(it == 1, NP // 2 - 1, it - 2)

            @pl.when(it == 1)
            def _():
                wait("zw4", [c_ax(1)])

            @pl.when(it > 1)
            def _():
                @pl.when(it + 1 < NP // 2)
                def _():
                    start(c_w(it + 1))
                for k in range(2):
                    if wos[k + 1] > wos[k]:
                        @pl.when(it == NB // 2 - 2 + k)
                        def _():
                            start(c_wo[wos[k]:wos[k + 1]])
                wait("zwl", c_w(c))

            def mid():
                @pl.when(it == 1)
                def _():
                    wait("zw4", [c_ax(2)])
                    start([c_mem, c_bx0] + c_w(2))
            a_body(2 * it, [2 * c, 2 * c + 1], mid)
            return carry
        lax.fori_loop(1, NB // 2, a_iter, 0)
        PD = NP - 4
        wait("zw5", c_w(NB // 2 - 2) + c_w(NB // 2 - 1) + [c_mem, c_bx0])
        start(c_wo[wos[2]:])
        late = attn_tasks(1)
        late_w = [t for p in range(PD, NP) for t in prep_tasks(p)]

        def step(s, hb, before_out=None):
            rows = pl.ds(s * SEG if isinstance(s, int) else pl.multiple_of(s * SEG, SEG), SEG)
            h_s[hb, M:L, :] = bx[rows, :].astype(F32)
            st = {}

            def proj(p, from_raw=False):
                if from_raw:
                    w = jnp.concatenate([raw[j, ds(p, PW), :] for j in range(3)], axis=0)
                    qkv = lax.dot_general(h_s[hb], w, NT, preferred_element_type=F32)
                else:
                    qkv = jnp.dot(h_s[hb], pltpu.bitcast(w3[p], BF16), preferred_element_type=F32)
                st[p] = dict(q=qkv[:, 0:PW], kb=_blockdiag(qkv[:, PW:2 * PW]),
                             vb=_blockdiag(qkv[:, 2 * PW:3 * PW]))

            def score(p):
                sc = lax.dot_general(st[p]["q"], st[p]["kb"], NT, preferred_element_type=F32)
                st[p]["p"] = _softmax_pair(sc)

            def pv(p):
                o_s[:, p * PW:(p + 1) * PW] = jnp.dot(st[p]["p"], st[p]["vb"], preferred_element_type=F32)

            acc = [None]

            def outp(ch):
                if before_out is not None:
                    before_out(ch)
                cs = slice(ch * ochunk * PW, (ch + 1) * ochunk * PW)
                r = jnp.dot(o_s[:, cs], wo[cs, :], preferred_element_type=F32)
                acc[0] = r if acc[0] is None else acc[0] + r

            nch = NP // ochunk
            done = 0
            fst = before_out is not None
            l1, l2 = (lag1, lag2) if not fst else lag0
            for t in range(NP + l2):
                if t < NP:
                    if fst and xp and t >= PD:
                        proj(t, True)
                    else:
                        proj(t)
                if fst:
                    for task in late[t * len(late) // nl:(t + 1) * len(late) // nl]:
                        task()
                    if not xp and t >= w0:
                        u = t - w0
                        for task in late_w[u * len(late_w) // (PD - w0):(u + 1) * len(late_w) // (PD - w0)]:
                            task()
                if 0 <= t - l1 < NP:
                    score(t - l1)
                if t >= NP and done < nch - 1 and not fst:
                    outp(done)
                    done += 1
                if fst and t >= NP:
                    ot = out_tasks(NB - 1, 1)
                    for task in ot[(t - NP) * len(ot) // l2:(t - NP + 1) * len(ot) // l2]:
                        task()
                if 0 <= t - l2 < NP:
                    pv(t - l2)
            if fst and xp:
                for task in late_w:
                    task()
            hn = (hb + 1) % UN if before_out is None else 0
            if omode == "k" or before_out is not None:
                while done < nch:
                    outp(done)
                    done += 1
                out = acc[0]
                h_s[hn, 0:M, :] = out[0:M]
                outb[rows, :] = out[M:L].astype(BF16)
            else:
                cs = slice(done * ochunk * PW, NP * PW)
                for n in range(LT):
                    ns = slice(n * 128, (n + 1) * 128)
                    out = acc[0][:, ns] + jnp.dot(o_s[:, cs], wo[cs, ns], preferred_element_type=F32)
                    h_s[hn, 0:M, ns] = out[0:M]
                    outb[rows, ns] = out[M:L].astype(BF16)

        h_s[0, 0:M, :] = mem[...].astype(F32)

        def wait_wo(ch):
            r0 = ch * ochunk * PW
            if r0 == 0:
                wait("zwo", c_wo)
                c_bx1.start()
        step(0, 0, wait_wo)
        c_outa = cp(outa, out_hbm.at[:, pl.ds(0, D)], sem_o.at[0])
        c_outa.start()

        def c_outb(r0, n):
            r = pl.ds(r0, n)
            return cp(outb.at[r, :], out_hbm.at[r, pl.ds(D, D)], sem_o.at[1])
        c_outb(0, SEG).start()

        def b_iter(it, carry):
            s0 = 1 + it * UN

            @pl.when(it == 1)
            def _():
                c_bx1.wait()
            for u in range(UN):
                step(s0 + u, u)
            c_outb(pl.multiple_of(s0 * SEG, SEG), UN * SEG).start()
            return carry
        lax.fori_loop(0, NIT, b_iter, 0)
        wait("zend", [c_outa, c_outb(0, SEG + NIT * UN * SEG)])

    V = pltpu.VMEM
    DMA = pltpu.SemaphoreType.DMA
    f = pl.pallas_call(
        kern,
        out_shape=jax.ShapeDtypeStruct((S, 2 * D), BF16),
        in_specs=[pl.BlockSpec(memory_space=pl.ANY)] * 9,
        out_specs=pl.BlockSpec(memory_space=pl.ANY),
        scratch_shapes=[
            V((S, D), BF16), V((3, D, D), BF16), V((D, D), BF16), V((LT, D, 128), F32),
            V((3 * D // 2, D), U32), V((D // 2, D), U32), V((2, LT, TB, 128), F32),
            V((2, 2 * LT, HALO + TB, 128), F32), V((2, TB, D), F32), V((S, D), BF16),
            V((S, D), BF16), V((M, D), BF16), V((3, H * DH, D), BF16), V((NP, D // 2, 3 * PW), U32),
            V((H * DH, D), BF16), V((UN, L, D), F32), V((L, H * DH), F32), V((S, D), BF16),
            DMA((4,)), DMA((3,)), DMA((NP // 2, 3)), DMA((3,)), DMA((WC,)), DMA((2,)),
        ] + [V((8 + LT * RC, 128), F32)] * 4,
        name="kf",
        compiler_params=pltpu.CompilerParams(vmem_limit_bytes=120 * 1024 * 1024))

    def fn(A_x, A_wqkv, A_wo, B_x, B_mem0, B_Wq, B_Wk, B_Wv, B_Wo):
        t = lambda w: w.transpose(1, 2, 0).reshape(H * DH, D)
        out = f(A_x.reshape(S, D), A_wqkv, A_wo, B_x.reshape(S, D), B_mem0.reshape(M, D),
                t(B_Wq), t(B_Wk), t(B_Wv), B_Wo.reshape(H * DH, D))
        return out.reshape(1, S, 2 * D)
    return fn


def pallas_concat_heads__sliding_local_dilated__memory_aug_recurrent_mem_tr__prompt_kernel(
    A_x, A_wqkv, A_wo, B_x, B_mem0, B_Wq, B_Wk, B_Wv, B_Wo, B_seg_len,
):
    assert B_seg_len == SEG
    return make(UN=3, omode='n', wos=[0, 1, 2])(A_x, A_wqkv, A_wo, B_x, B_mem0, B_Wq, B_Wk, B_Wv, B_Wo)
```

```python
import functools

import jax
import jax.numpy as jnp
from jax import lax
from jax.experimental import pallas as pl
from jax.experimental.pallas import tpu as pltpu

F32, BF16, U32 = jnp.float32, jnp.bfloat16, jnp.uint32
NT = (((1,), (1,)), ((), ()))
MASKED = -1000000000.0

S, D = 2048, 640
LT = D // 128

AH, AD, AW, ADIL = 32, 20, 8, 2
HALO = 16
TB = 128
NB = S // TB
RC = 8

H, DH, M, SEG = 32, 192, 8, 32
L = M + SEG
NP = H // 2
PW = 2 * DH
NSEG = S // SEG
UN = 3
NCH = NP // 2
WOC = 4


def _ds(i, n):
    return pl.ds(i * n if isinstance(i, int) else pl.multiple_of(i * n, n), n)


def _dot(a, b):
    return jnp.dot(a, b, preferred_element_type=F32)


def _share(tasks, k, n):
    return tasks[k * len(tasks) // n:(k + 1) * len(tasks) // n]


def _run(tasks):
    for task in tasks:
        task()


def _block_diag(t):
    lane = lax.broadcasted_iota(jnp.int32, (L, 128), 1)
    zero = jnp.zeros((L, 128), F32)
    t0, t1, t2 = t[:, 0:128], t[:, 128:256], t[:, 256:384]
    top = jnp.concatenate([t0, jnp.where(lane < 64, t1, 0.0), zero], axis=1)
    bot = jnp.concatenate([zero, jnp.where(lane >= 64, t1, 0.0), t2], axis=1)
    return jnp.concatenate([top, bot], axis=0).astype(BF16)


def _kernel(ax_hbm, awqkv_hbm, awo_hbm, bx_hbm, mem_hbm, wq_hbm, wk_hbm, wv_hbm, wo_hbm,
            out_hbm,
            ax, awqkv, awo, tmp, wqkv_p, wo_p, q_s, kv_s, oa_s, outa,
            bx, mem, raw, w3, wo, h_s, o_s, outb, order0, order1, order2,
            sem_a, sem_x, sem_w, sem_b, sem_wo, sem_o):
    cp = pltpu.make_async_copy

    def rows_copy(src, dst, r0, r1, sem):
        return cp(src.at[pl.ds(r0, r1 - r0), :], dst.at[pl.ds(r0, r1 - r0), :], sem)

    c_wqkv = [cp(awqkv_hbm.at[:, pl.ds(j * D, D)], awqkv.at[j], sem_a.at[j]) for j in range(3)]
    c_awo = cp(awo_hbm, awo, sem_a.at[3])
    x_cuts = (0, 2 * TB, 4 * TB, S)
    c_ax = [rows_copy(ax_hbm, ax, x_cuts[c], x_cuts[c + 1], sem_x.at[c]) for c in range(3)]
    c_mem = cp(mem_hbm, mem, sem_b.at[0])
    c_bx0 = rows_copy(bx_hbm, bx, 0, (1 + UN) * SEG, sem_b.at[1])
    c_bx1 = rows_copy(bx_hbm, bx, (1 + UN) * SEG, S, sem_b.at[2])
    wo_rows = H * DH // WOC
    c_wo = [rows_copy(wo_hbm, wo, c * wo_rows, (c + 1) * wo_rows, sem_wo.at[c]) for c in range(WOC)]
    c_outa = cp(outa, out_hbm.at[:, pl.ds(0, D)], sem_o.at[0])

    def c_w(c):
        return [cp(w.at[_ds(c, 2 * PW), :], raw.at[j, _ds(c, 2 * PW), :], sem_w.at[c, j])
                for j, w in enumerate((wq_hbm, wk_hbm, wv_hbm))]

    def c_outb(r0, n):
        return cp(outb.at[pl.ds(r0, n), :], out_hbm.at[pl.ds(r0, n), pl.ds(D, D)], sem_o.at[1])

    def start(copies):
        for c in copies:
            c.start()

    def wait(copies):
        for c in copies:
            c.wait()

    def permute_rows(dst, base):
        for d in range(AD):
            for t in range(LT):
                dst[pl.ds((base + d * AH) // 2, AH // 2), t * 128:(t + 1) * 128] = pltpu.bitcast(
                    tmp[t, pl.ds(d, AH, stride=AD), :].astype(BF16), U32)

    def prep_wqkv(j):
        for t in range(LT):
            tmp[t] = awqkv[j, t * 128:(t + 1) * 128, :].astype(F32).T
        permute_rows(wqkv_p, j * D)

    def prep_wo():
        for t in range(LT):
            tmp[t] = awo[:, t * 128:(t + 1) * 128].astype(F32)
        permute_rows(wo_p, 0)

    def a_proj(i, b, j):
        w = pltpu.bitcast(wqkv_p[j * D // 2:(j + 1) * D // 2, :], BF16)
        r = lax.dot_general(ax[_ds(i, TB), :], w, NT, preferred_element_type=F32)
        for t in range(LT):
            rt = r[:, t * 128:(t + 1) * 128]
            if j == 0:
                q_s[b, t] = rt
                continue
            c = (j - 1) * LT + t
            kv_s[b, c, HALO:HALO + TB, :] = rt
            if isinstance(i, int) and i == 0:
                kv_s[b, c, 0:HALO, :] = jnp.broadcast_to(rt[0:1, :], (HALO, 128))
            else:
                kv_s[b, c, 0:HALO, :] = kv_s[1 - b, c, TB:TB + HALO, :]

    def a_attention(b, first_block=False):
        state = {}

        def window(c, r0, w):
            lo = HALO + r0 - ADIL * w
            return kv_s[b, c, lo:lo + RC, :]

        def logits(r0):
            q = [q_s[b, t, r0:r0 + RC, :] for t in range(LT)]
            state[r0] = []
            for w in range(AW):
                a = q[0] * window(0, r0, w)
                for t in range(1, LT):
                    a = a + q[t] * window(t, r0, w)
                state[r0].append(a + pltpu.roll(a, 2 * AH, 1))

        def fold(r0):
            state[r0] = [a + pltpu.roll(a, AH, 1) for a in state[r0]]

        def mix(r0):
            lg = []
            for w, a in enumerate(state.pop(r0)):
                a = a * (AD ** -0.5)
                if first_block and r0 < ADIL * w:
                    pos = lax.broadcasted_iota(jnp.int32, (RC, 128), 0) + r0
                    a = jnp.where(pos >= ADIL * w, a, MASKED)
                lg.append(a)
            m = functools.reduce(jnp.maximum, lg)
            e = [jnp.exp(a - m) for a in lg]
            inv = 1.0 / functools.reduce(jnp.add, e)
            p = [x * inv for x in e]
            for t in range(LT):
                o = p[0] * window(LT + t, r0, 0)
                for w in range(1, AW):
                    o = o + p[w] * window(LT + t, r0, w)
                oa_s[b, r0:r0 + RC, t * 128:(t + 1) * 128] = o

        n = TB // RC
        return [functools.partial(f, (k - lag) * RC) for k in range(n + 2)
                for lag, f in enumerate((logits, fold, mix)) if 0 <= k - lag < n]

    def a_out(i, b):
        outa[_ds(i, TB), :] = _dot(oa_s[b], pltpu.bitcast(wo_p[...], BF16)).astype(BF16)

    def a_stage(i, b, extra=(), first_block=False):
        side = a_attention(1 - b, first_block) + list(extra)
        for j in range(3):
            a_proj(i, b, j)
            _run(_share(side, j, 3))
        a_out(i - 1, 1 - b)

    def w_prep(p, j):
        w3[p, :, j * PW:(j + 1) * PW] = pltpu.bitcast(raw[j, _ds(p, PW), :].T, U32)

    start([c_wqkv[0], c_ax[0], c_wqkv[1]])
    c_wqkv[0].wait()
    c_wqkv[2].start()
    prep_wqkv(0)
    wait([c_ax[0], c_wqkv[1]])
    start([c_awo, c_ax[1]])
    a_proj(0, 0, 0)
    prep_wqkv(1)
    c_wqkv[2].wait()
    c_ax[2].start()
    a_proj(0, 0, 1)
    prep_wqkv(2)
    a_proj(0, 0, 2)
    c_awo.wait()
    start(c_w(0))
    prep_wo()
    a_stage(1, 1, first_block=True)
    start(c_w(1))

    def a_step(it, carry):
        c = jnp.where(it == 1, NCH - 1, it - 2)

        @pl.when(it == 1)
        def _():
            c_ax[1].wait()

        @pl.when(it > 1)
        def _():
            @pl.when(it + 1 < NCH)
            def _():
                start(c_w(it + 1))
            for k in range(2):
                @pl.when(it == NB // 2 - 2 + k)
                def _():
                    c_wo[k].start()
            wait(c_w(c))

        preps = [functools.partial(w_prep, 2 * c + u, j) for j in range(3) for u in range(2)]
        a_stage(2 * it, 0, preps[:3])

        @pl.when(it == 1)
        def _():
            c_ax[2].wait()
            start([c_mem, c_bx0] + c_w(2))
        a_stage(2 * it + 1, 1, preps[3:])
        return carry

    lax.fori_loop(1, NB // 2, a_step, 0)
    wait(c_w(NCH - 2) + c_w(NCH - 1) + [c_mem, c_bx0])
    start(c_wo[2:])

    NK = 2 * M
    order = (order0, order1, order2)

    def segment(s, hb, peeled=False):
        h_s[hb, M:L, :] = bx[_ds(s, SEG), :].astype(F32)
        row = lax.broadcasted_iota(jnp.int32, (L, 2 * L), 0)
        col = lax.broadcasted_iota(jnp.int32, (L, 2 * L), 1)
        head0 = col < L
        visible = (row < M) | (row >= jnp.where(head0, col, col - L))
        st = [dict() for _ in range(NP)]

        def proj(p):
            qkv = _dot(h_s[hb], pltpu.bitcast(w3[p], BF16))
            v = qkv[:, 2 * PW:3 * PW]
            st[p].update(q=qkv[:, 0:PW], k=_block_diag(qkv[:, PW:2 * PW]), v=_block_diag(v))
            if not peeled:
                rest = v[NK:NK + 8] + v[NK + 8:NK + 16] + v[NK + 16:L]
                st[p].update(v_near=v[0:NK], v_rest=jnp.sum(rest, axis=0, keepdims=True))

        def score(p):
            sc = lax.dot_general(st[p]["q"], st[p]["k"], NT, preferred_element_type=F32)
            sc = jnp.where(visible, sc * (DH ** -0.5), MASKED)
            m0 = jnp.max(jnp.where(head0, sc, -jnp.inf), axis=1, keepdims=True)
            m1 = jnp.max(jnp.where(head0, -jnp.inf, sc), axis=1, keepdims=True)
            st[p]["s"] = sc - jnp.where(head0, m0, m1)

        def normalize(p):
            e = jnp.exp(st[p]["s"])
            l0 = jnp.sum(jnp.where(head0, e, 0.0), axis=1, keepdims=True)
            l1 = jnp.sum(jnp.where(head0, 0.0, e), axis=1, keepdims=True)
            st[p]["p"] = e / jnp.where(head0, l0, l1)

        def pv_near(p):
            pr = st[p]["p"][M:NK]
            low = lax.broadcasted_iota(jnp.int32, (8, 128), 1) < 64
            key = lax.broadcasted_iota(jnp.int32, (8, 2 * L), 1)
            acc = [None] * 3
            for j in range(NK + 1):
                a, b = [jnp.broadcast_to(
                    jnp.sum(jnp.where(key == c, pr, 0.0), axis=1, keepdims=True), (8, 128))
                    for c in (j, L + j)]
                vj = st[p]["v_near"][j:j + 1] if j < NK else st[p]["v_rest"]
                for t, w in enumerate((a, jnp.where(low, a, b), b)):
                    term = w * vj[:, t * 128:(t + 1) * 128]
                    acc[t] = term if j == 0 else acc[t] + term
            for t in range(3):
                o_s[M:NK, p * PW + t * 128:p * PW + (t + 1) * 128] = acc[t]
                order[p % 3][8 + 8 * t:16 + 8 * t, :] = acc[t]

        def pv(p):
            pr = st[p]["p"]
            cols = slice(p * PW, (p + 1) * PW)
            if peeled:
                o_s[:, cols] = _dot(pr, st[p]["v"])
                return
            zero = pl.multiple_of(lax.shift_right_logical(s, 16) * 8, 8)
            order[p % 3][0:M, 0:2 * L] = pr[0:M]
            pr = jnp.concatenate([order[p % 3][pl.ds(zero, M), 0:2 * L], pr[NK:L]], axis=0)
            r = _dot(pr, st[p]["v"])
            o_s[0:M, cols] = r[0:M]
            o_s[NK:L, cols] = r[M:]

        def out_chunk(acc, c):
            cols = slice(c * 2 * PW, (c + 1) * 2 * PW)
            r = _dot(o_s[:, cols], wo[cols, :])
            return r if acc is None else acc + r

        if peeled:
            lag_s, lag_n, lag_pv = 2, 2, 6
            last_attention = a_attention(1)
            last_preps = [functools.partial(w_prep, p, j) for p in range(NP - 4, NP) for j in range(3)]
        else:
            lag_s, lag_n, lag_pv = 1, 2, 4
        acc = None
        for t in range(NP + lag_pv):
            if t < NP:
                proj(t)
            if peeled:
                _run(_share(last_attention, t, 6) + _share(last_preps, t, NP - 4))
                if t == NP + lag_pv - 1:
                    a_out(NB - 1, 1)
            elif t >= NP:
                acc = out_chunk(acc, t - NP)
            if lag_pv <= t:
                pv(t - lag_pv)
            if not peeled:
                if 0 <= t - lag_n < NP:
                    normalize(t - lag_n)
                if 0 <= t - lag_n - 1 < NP:
                    pv_near(t - lag_n - 1)
            if 0 <= t - lag_s < NP:
                score(t - lag_s)
                if peeled:
                    normalize(t - lag_s)
        if peeled:
            wait(c_wo)
            c_bx1.start()
            for c in range(NCH):
                acc = out_chunk(acc, c)
            h_s[0, 0:M, :] = acc[0:M]
            outb[0:SEG, :] = acc[M:L].astype(BF16)
            return
        k0 = lag_pv * 2 * PW
        for n in range(LT):
            lanes = slice(n * 128, (n + 1) * 128)
            out = acc[:, lanes] + _dot(o_s[:, k0:], wo[k0:, lanes])
            h_s[(hb + 1) % UN, 0:M, lanes] = out[0:M]
            outb[_ds(s, SEG), lanes] = out[M:L].astype(BF16)

    h_s[0, 0:M, :] = mem[...].astype(F32)
    segment(0, 0, peeled=True)
    c_outa.start()
    c_outb(0, SEG).start()

    def b_step(it, carry):
        @pl.when(it == 1)
        def _():
            c_bx1.wait()
        s0 = 1 + it * UN
        for u in range(UN):
            segment(s0 + u, u)
        c_outb(pl.multiple_of(s0 * SEG, SEG), UN * SEG).start()
        return carry

    lax.fori_loop(0, (NSEG - 1) // UN, b_step, 0)
    c_outa.wait()
    c_outb(0, S).wait()


def pallas_concat_heads__sliding_local_dilated__memory_aug_recurrent_mem_tr__prompt_kernel(
    A_x, A_wqkv, A_wo, B_x, B_mem0, B_Wq, B_Wk, B_Wv, B_Wo, B_seg_len,
):
    assert B_seg_len == SEG and (NSEG - 1) % UN == 0
    assert A_x.shape == B_x.shape == (1, S, D) and B_mem0.shape == (1, M, D)
    assert B_Wq.shape == B_Wk.shape == B_Wv.shape == (D, H, DH) and B_Wo.shape == (H, DH, D)
    vmem, dma = pltpu.VMEM, pltpu.SemaphoreType.DMA
    call = pl.pallas_call(
        _kernel,
        out_shape=jax.ShapeDtypeStruct((S, 2 * D), BF16),
        in_specs=[pl.BlockSpec(memory_space=pl.ANY)] * 9,
        out_specs=pl.BlockSpec(memory_space=pl.ANY),
        scratch_shapes=[
            vmem((S, D), BF16),
            vmem((3, D, D), BF16),
            vmem((D, D), BF16),
            vmem((LT, D, 128), F32),
            vmem((3 * D // 2, D), U32),
            vmem((D // 2, D), U32),
            vmem((2, LT, TB, 128), F32),
            vmem((2, 2 * LT, HALO + TB, 128), F32),
            vmem((2, TB, D), F32),
            vmem((S, D), BF16),
            vmem((S, D), BF16),
            vmem((M, D), BF16),
            vmem((3, H * DH, D), BF16),
            vmem((NP, D // 2, 3 * PW), U32),
            vmem((H * DH, D), BF16),
            vmem((UN, L, D), F32),
            vmem((L, H * DH), F32),
            vmem((S, D), BF16),
            vmem((32, 128), F32), vmem((32, 128), F32), vmem((32, 128), F32),
            dma((4,)), dma((3,)), dma((NCH, 3)), dma((3,)), dma((WOC,)), dma((2,)),
        ],
        compiler_params=pltpu.CompilerParams(vmem_limit_bytes=100 * 1024 * 1024),
        name="sliding_and_memory_attention",
    )

    def by_feature(w):
        return w.transpose(1, 2, 0).reshape(H * DH, D)

    out = call(A_x.reshape(S, D), A_wqkv, A_wo, B_x.reshape(S, D), B_mem0.reshape(M, D),
               by_feature(B_Wq), by_feature(B_Wk), by_feature(B_Wv), B_Wo.reshape(H * DH, D))
    return out.reshape(1, S, 2 * D)
```
